```python
import os as _os
_os.environ.setdefault("JAX_PLATFORMS", "cpu")
import jax
import jax.numpy as jnp

def _softmax(x, axis=-1):
    return jax.nn.softmax(x, axis=axis)
def _gelu(x):
    return jax.nn.gelu(x, approximate=True)
def _silu(x):
    return jax.nn.silu(x)
def _sigmoid(x):
    return jax.nn.sigmoid(x)
def _layernorm(x, axis=-1, eps=1e-5):
    m = jnp.mean(x, axis=axis, keepdims=True)
    v = jnp.var(x, axis=axis, keepdims=True)
    return (x - m) / jnp.sqrt(v + eps)
def _scatter_add(tgt, idx, src, axis=0):
    return tgt.at[idx].add(src)
def _segment_sum(src, seg, n):
    return jax.ops.segment_sum(src, seg, n)
class _Rng:
    def __init__(self, key):
        self._k = key
    def _next(self):
        self._k, sub = jax.random.split(self._k)
        return sub
    def normal(self, shape):
        return jax.random.normal(self._next(), shape, dtype=jnp.bfloat16)
    def randint(self, lo, hi, shape):
        return jax.random.randint(self._next(), shape, lo, hi, dtype=jnp.int32)
    def uniform(self, shape, lo=0.0, hi=1.0):
        return jax.random.uniform(self._next(), shape, jnp.bfloat16, lo, hi)
    def permutation(self, n):
        return jax.random.permutation(self._next(), n)


kernel_name = 'gated_mix__mha_block__mixer_s_mlp__prompt'

def setup_inputs():
    _rng = _Rng(jax.random.key(int.from_bytes(__import__("os").urandom(4), "little")))
    _w = (lambda a: (lambda t: t.astype(jnp.bfloat16) if jnp.issubdtype(t.dtype, jnp.floating) else t)(jnp.asarray(a)))
    def _A_setup():
        B, S, D, H = 1, 2048, 448, 16
        return {
            "x": _w((lambda *s: _rng.normal(s) * 0.05)(B, S, D)),
            "wqkv": _w((lambda *s: _rng.normal(s) * 0.8)(D, 3 * D)),
            "wo": _w((lambda *s: _rng.normal(s) * 0.05)(D, D)),
        }
    _A_in = _A_setup()

    def _B_setup():
        B, S, D, F = 1, 2048, 448, 1792
        return {
            "x":  _w((lambda *s: _rng.normal(s) * 0.05)(B, S, D)),
            "w1": _w((lambda *s: _rng.normal(s) * 0.2)(D, D) * (D ** -0.5)),
            "w2": _w((lambda *s: _rng.normal(s) * 0.2)(D, D) * (D ** -0.5)),
            "w3": _w((lambda *s: _rng.normal(s) * 0.2)(D, F) * (D ** -0.5)),
            "w4": _w((lambda *s: _rng.normal(s) * 0.2)(F, D) * (F ** -0.5)),
        }
    _B_in = _B_setup()

    return {
        "A_x": _A_in["x"],
        "A_wqkv": _A_in["wqkv"],
        "A_wo": _A_in["wo"],
        "B_x": _B_in["x"],
        "B_w1": _B_in["w1"],
        "B_w2": _B_in["w2"],
        "B_w3": _B_in["w3"],
        "B_w4": _B_in["w4"],
        "gate_w": _w((lambda *s: _rng.normal(s) * 0.05)(448) * 16.0),
    }

def reference(A_x, A_wqkv, A_wo, B_x, B_w1, B_w2, B_w3, B_w4, gate_w):
    def _A_ref(x, wqkv, wo):
        B, S, D = x.shape
        H = 16
        Dh = D // H
        qkv = (lambda x, *d: x.transpose(*d))((x @ wqkv).reshape(B, S, 3, H, Dh), 2, 0, 3, 1, 4)
        q, k, v = qkv[0], qkv[1], qkv[2]
        scores = jnp.einsum("bhqd,bhkd->bhqk", q, k) * (Dh ** -0.5)
        p = _softmax(scores, axis=-1)
        o = jnp.einsum("bhqk,bhkd->bhqd", p, v)
        return (lambda x, *d: x.transpose(*d))(o, 0, 2, 1, 3).reshape(B, S, D) @ wo

    def _B_ref(x, w1, w2, w3, w4):
        B, S, D = x.shape
        h = _gelu(_layernorm(x, axis=-1) @ w1)
        c = D // 4
        g0 = jnp.pad(h[:, :, 0*c:1*c], ((0, 0), (1, 0), (0, 0)))[:, :S, :]
        g1 = jnp.pad(h[:, :, 1*c:2*c], ((0, 0), (0, 1), (0, 0)))[:, 1:, :]
        g2 = jnp.pad(h[:, :, 2*c:3*c], ((0, 0), (2, 0), (0, 0)))[:, :S, :]
        g3 = jnp.pad(h[:, :, 3*c:   ], ((0, 0), (0, 2), (0, 0)))[:, 2:, :]
        hs = jnp.concatenate([g0, g1, g2, g3], axis=-1) @ w2
        x1 = x + hs
        h2 = _gelu(_layernorm(x1, axis=-1) @ w3) @ w4
        return x1 + h2

    x = A_x
    g = _sigmoid((x * gate_w).sum(-1, keepdims=True))
    a = _A_ref(x, A_wqkv, A_wo)
    b = _B_ref(x, B_w1, B_w2, B_w3, B_w4)
    return g * a + (1 - g) * b
```

```python
import functools
import math

import jax
import jax.numpy as jnp
from jax import lax
import jax.experimental.pallas as pl
import jax.experimental.pallas.tpu as pltpu

F32 = jnp.float32
BF16 = jnp.bfloat16

H = 16
HG = 4
NG = H // HG
HP = 32
TQ = 512
CK = 128
EPS = 1e-5
HALO = 128


def _dot(a, b):
    return jnp.dot(a, b, preferred_element_type=F32)


def _gelu(x):
    c = math.sqrt(2.0 / math.pi)
    return 0.5 * x * (1.0 + jnp.tanh(c * (x + 0.044715 * (x * x * x))))


def _layernorm_t(x):
    m = jnp.mean(x, axis=0, keepdims=True)
    xc = x - m
    v = jnp.mean(xc * xc, axis=0, keepdims=True)
    return xc * lax.rsqrt(v + EPS)


def _kernel(xt_ref, wqkv_ref, wo_ref, w1_ref, w2_ref, w3_ref, w4t_ref, gw_ref,
            out_ref,
            wqkvt_s, wot_s, w1t_s, w2t_s, w3t_s, gw_s, tmp_s, tmp2_s,
            qt_s, k_s, vt_s, ot_s, s_a, s_b, m_a, m_b, h_s,
            *, S, D, FF):
    DH = D // H
    GW = HG * DH
    NQ = S // TQ
    NC = S // CK
    qscale = (DH ** -0.5) * math.log2(math.e)

    wqkvt_s[...] = wqkv_ref[...].T
    w1t_s[...] = w1_ref[...].T
    w2t_s[...] = w2_ref[...].T
    w3t_s[...] = w3_ref[...].T
    tmp2_s[...] = jnp.zeros_like(tmp2_s)
    tmp_s[...] = wo_ref[...].astype(F32)
    for h in range(H):
        tmp2_s[h * HP:h * HP + DH, :] = tmp_s[h * DH:(h + 1) * DH, :]
    wot_s[...] = tmp2_s[...].astype(BF16).T
    gw_s[...] = jnp.broadcast_to(gw_ref[...].astype(F32), (128, D)).T

    h_s[:, 0:HALO] = jnp.zeros((D, HALO), BF16)
    h_s[:, HALO + S:HALO + S + HALO] = jnp.zeros((D, HALO), BF16)

    zpad = jnp.zeros((128 - GW, TQ), BF16)
    rowv = lax.broadcasted_iota(jnp.int32, (HP - DH, TQ), 0)
    vtail = jnp.where(rowv == 0, 1.0, 0.0).astype(F32)

    def proj_body(i, carry):
        c0 = pl.multiple_of(i * TQ, TQ)
        xc = xt_ref[:, pl.ds(c0, TQ)]
        for g in range(NG):
            q = _dot(wqkvt_s[g * GW:(g + 1) * GW, :], xc) * qscale
            qt_s[i, g] = jnp.concatenate([q.astype(BF16), zpad], axis=0)
        for g in range(NG):
            kt = _dot(wqkvt_s[D + g * GW:D + (g + 1) * GW, :], xc)
            kt = jnp.concatenate([kt.astype(BF16), zpad], axis=0)
            k_s[g, pl.ds(c0, TQ), :] = kt.T
        for g in range(NG):
            vt = _dot(wqkvt_s[2 * D + g * GW:2 * D + (g + 1) * GW, :], xc)
            for j in range(HG):
                vh = jnp.concatenate([vt[j * DH:(j + 1) * DH], vtail], axis=0).astype(BF16)
                for c in range(TQ // CK):
                    vt_s[i * (TQ // CK) + c, (g * HG + j) * HP:(g * HG + j + 1) * HP, :] = vh[:, c * CK:(c + 1) * CK]
        ln = _layernorm_t(xc.astype(F32)).astype(BF16)
        for g in range(4):
            hh = _gelu(_dot(w1t_s[g * GW:(g + 1) * GW, :], ln))
            h_s[g * GW:(g + 1) * GW, pl.ds(c0 + HALO, TQ)] = hh.astype(BF16)
        return carry

    lax.fori_loop(0, NQ, proj_body, 0)

    sb = (s_a, s_b)
    mb = (m_a, m_b)
    row = lax.broadcasted_iota(jnp.int32, (128, TQ), 0)

    def step(nxt, cur, par):
        if nxt is not None:
            qi1, g1, j1 = nxt
            qg = qt_s[qi1, g1]
            qg = jnp.where((row >= DH * j1) & (row < DH * (j1 + 1)), qg, jnp.zeros_like(qg))
            mx = None
        if cur is not None:
            qi, g, j = cur
            hrow = pl.multiple_of((g * HG + j) * HP, HP)
            m = mb[par][...]
            acc = None
        for c in range(NC):
            sl = pl.ds(c * CK, CK)
            if nxt is not None:
                s = _dot(k_s[g1, sl, :], qg)
                sb[1 - par][sl, :] = s
                cm = jnp.max(s.reshape(CK // 8, 8, TQ), axis=0)
                mx = cm if mx is None else jnp.maximum(mx, cm)
            if cur is not None:
                p = jnp.exp2(sb[par][sl, :] - m).astype(BF16)
                o = _dot(vt_s[c, pl.ds(hrow, HP), :], p)
                acc = o if acc is None else acc + o
        if nxt is not None:
            mb[1 - par][...] = jnp.max(mx, axis=0, keepdims=True)
        if cur is not None:
            inv = 1.0 / acc[DH:DH + 1, :]
            ot_s[qi, pl.ds(hrow, HP), :] = (acc * inv).astype(BF16)

    step((0, 0, 0), None, 1)

    def attn_body(i, carry):
        qi = i // NG
        g = i % NG
        i1 = i + 1
        for j in range(HG):
            nxt = (qi, g, j + 1) if j + 1 < HG else (i1 // NG, i1 % NG, 0)
            step(nxt, (qi, g, j), j % 2)
        return carry

    nblk = NQ * NG
    lax.fori_loop(0, nblk - 1, attn_body, 0)
    for j in range(HG):
        nxt = (NQ - 1, NG - 1, j + 1) if j + 1 < HG else None
        step(nxt, (NQ - 1, NG - 1, j), j % 2)

    C = D // 4
    FC = 256

    def mix_body(i, carry):
        c0 = pl.multiple_of(i * TQ, TQ)
        x32 = xt_ref[:, pl.ds(c0, TQ)].astype(F32)
        parts = []
        for g, sh in enumerate((-1, 1, -2, 2)):
            hw = h_s[g * C:(g + 1) * C, pl.ds(c0, TQ + 2 * HALO)]
            parts.append(hw[:, HALO + sh:HALO + sh + TQ])
        hs = jnp.concatenate(parts, axis=0)
        x1 = x32 + _dot(w2t_s[...], hs)
        ln = _layernorm_t(x1).astype(BF16)
        b = x1
        for f in range(FF // FC):
            gch = _gelu(_dot(w3t_s[f * FC:(f + 1) * FC, :], ln))
            b = b + _dot(w4t_ref[:, f * FC:(f + 1) * FC], gch.astype(BF16))
        a = _dot(wot_s[...], ot_s[i])
        gw = jnp.concatenate([gw_s[...]] * (TQ // 128), axis=1)
        gate = jax.nn.sigmoid(jnp.sum(x32 * gw, axis=0, keepdims=True))
        out_ref[:, pl.ds(c0, TQ)] = (gate * a + (1.0 - gate) * b).astype(out_ref.dtype)
        return carry

    lax.fori_loop(0, NQ, mix_body, 0)


@jax.jit
def pallas_gated_mix__mha_block__mixer_s_mlp__prompt_kernel(
    A_x: jax.Array,
    A_wqkv: jax.Array,
    A_wo: jax.Array,
    B_x: jax.Array,
    B_w1: jax.Array,
    B_w2: jax.Array,
    B_w3: jax.Array,
    B_w4: jax.Array,
    gate_w: jax.Array,
):
    B, S, D = A_x.shape
    assert B == 1
    FF = B_w3.shape[1]
    xt = A_x.reshape(S, D).T
    w4t = B_w4.T
    gw = gate_w.reshape(1, D)

    scratch = [
        pltpu.VMEM((3 * D, D), BF16),
        pltpu.VMEM((D, H * HP), BF16),
        pltpu.VMEM((D, D), BF16),
        pltpu.VMEM((D, D), BF16),
        pltpu.VMEM((FF, D), BF16),
        pltpu.VMEM((D, 128), F32),
        pltpu.VMEM((D, D), F32),
        pltpu.VMEM((H * HP, D), F32),
        pltpu.VMEM((S // TQ, NG, 128, TQ), BF16),
        pltpu.VMEM((NG, S, 128), BF16),
        pltpu.VMEM((S // CK, H * HP, CK), BF16),
        pltpu.VMEM((S // TQ, H * HP, TQ), BF16),
        pltpu.VMEM((S, TQ), F32),
        pltpu.VMEM((S, TQ), F32),
        pltpu.VMEM((1, TQ), F32),
        pltpu.VMEM((1, TQ), F32),
        pltpu.VMEM((D, S + 2 * HALO), BF16),
    ]
    out = pl.pallas_call(
        functools.partial(_kernel, S=S, D=D, FF=FF),
        out_shape=jax.ShapeDtypeStruct((D, S), A_x.dtype),
        scratch_shapes=scratch,
        compiler_params=pltpu.CompilerParams(vmem_limit_bytes=100 * 1024 * 1024),
        name="gated_mix",
    )(xt, A_wqkv, A_wo, B_w1, B_w2, B_w3, w4t, gw)
    return out.T.reshape(B, S, D)
```

```python
import functools
import math

import jax
import jax.numpy as jnp
from jax import lax
import jax.experimental.pallas as pl
import jax.experimental.pallas.tpu as pltpu

F32 = jnp.float32
BF16 = jnp.bfloat16

H = 16
HG = 4
NG = H // HG
HP = 32
TQ = 512
CK = 128
EPS = 1e-5
HALO = 128
UG = 2
NOS = 4

OPT = dict(
    dma0="wv,x0,x1,wk,x2,x3,wq,w1,gw", dma1="wo,w2,w3,w4",
    plan="q0,q1|h0@3,h1@9,a|b|b|b|b|b|b,b|c|c@2,c@5,c@8,c@11,c@14,c",
)

_TN = (((0,), (0,)), ((), ()))


def _dot(a, b):
    return jnp.dot(a, b, preferred_element_type=F32)


def _dot_tn(a, b):
    return lax.dot_general(a, b, _TN, preferred_element_type=F32)


def _gelu(x):
    c = math.sqrt(2.0 / math.pi)
    return 0.5 * x * (1.0 + jnp.tanh(c * (x + 0.044715 * (x * x * x))))


def _ln_stats(x):
    n = x.shape[0]
    p = x[0:1, :]
    d = x - p
    s1 = jnp.sum(d, axis=0, keepdims=True) * (1.0 / n)
    s2 = jnp.sum(d * d, axis=0, keepdims=True) * (1.0 / n)
    v = jnp.maximum(s2 - s1 * s1, 0.0)
    r = lax.rsqrt(v + EPS)
    return r, (p + s1) * r


def _kernel(xt_hbm, wqkv_hbm, wo_hbm, w1_hbm, w2_hbm, w3_hbm, w4t_hbm, gw_hbm,
            out_hbm,
            gw_ref, xt_s, wqkv_s, w1_s, w2_s, wo_s, w3_s, w4t_s, out_s, sem_in, sem_x, sem_out,
            wkvt_s, wqt_s, wot_s, gw_s,
            qt_s, k_s, vt_s, ot_s, s_a, s_b, m_a, m_b, h_s, g_s, bb_s, gate_s,
            *, S, D, FF):
    DH = D // H
    GW = HG * DH
    NQ = S // TQ
    NC = S // CK
    qscale = (DH ** -0.5) * math.log2(math.e)
    NIT = NQ * NG // UG
    TB = S // NIT
    RO = D // NOS
    KLO = (D // 128) * 128
    C = D // 4

    def out_copy(i, r):
        return pltpu.make_async_copy(out_s.at[i, pl.ds(r * RO, RO)],
                                     out_hbm.at[pl.ds(r * RO, RO), pl.ds(i * TQ, TQ)],
                                     sem_out.at[i * NOS + r])

    def col_copy(src, dst, lo, hi, sem):
        return pltpu.make_async_copy(src.at[:, lo:hi], dst.at[:, lo:hi], sem)

    cp = dict(
        wk=col_copy(wqkv_hbm, wqkv_s, KLO, 2 * D, sem_in.at[0]),
        wv=col_copy(wqkv_hbm, wqkv_s, 2 * D, 3 * D, sem_in.at[1]),
        wq=col_copy(wqkv_hbm, wqkv_s, 0, KLO, sem_in.at[2]),
        w1=pltpu.make_async_copy(w1_hbm, w1_s, sem_in.at[3]),
        w3=pltpu.make_async_copy(w3_hbm, w3_s, sem_in.at[4]),
        w2=pltpu.make_async_copy(w2_hbm, w2_s, sem_in.at[5]),
        wo=pltpu.make_async_copy(wo_hbm, wo_s, sem_in.at[6]),
        w4=pltpu.make_async_copy(w4t_hbm, w4t_s, sem_in.at[7]),
        gw=pltpu.make_async_copy(gw_hbm, gw_ref, sem_in.at[8]),
    )
    for i in range(NQ):
        cp["x%d" % i] = col_copy(xt_hbm, xt_s, i * TQ, (i + 1) * TQ, sem_x.at[i])

    for name in OPT["dma0"].split(","):
        cp[name].start()
    h_s[:, 0:HALO] = jnp.zeros((D, HALO), BF16)
    xt_s[:, S:S + HALO] = jnp.zeros((D, HALO), BF16)
    for ref in (s_a, s_b):
        ref[0:8, :] = jnp.zeros((8, TQ), F32)
    for ref in (m_a, m_b):
        ref[...] = jnp.zeros_like(ref)
    for u in range(UG):
        qt_s[u, GW:128, :] = jnp.zeros((128 - GW, TQ), BF16)

    zpad = jnp.zeros((128 - GW, TQ), BF16)
    rowv = lax.broadcasted_iota(jnp.int32, (HP - DH, TQ), 0)
    vtail = jnp.where(rowv == 0, 1.0, 0.0).astype(F32)
    koff = D - KLO
    voff = 2 * D - KLO

    def proj_k(i):
        xc = xt_s[:, i * TQ:(i + 1) * TQ]
        for g in range(NG):
            kt = _dot(wkvt_s[koff + g * GW:koff + (g + 1) * GW, :], xc)
            kt = jnp.concatenate([kt.astype(BF16), zpad], axis=0)
            k_s[g, i * TQ:(i + 1) * TQ, :] = kt.T

    def proj_v(i):
        xc = xt_s[:, i * TQ:(i + 1) * TQ]
        for g in range(NG):
            vt = _dot(wkvt_s[voff + g * GW:voff + (g + 1) * GW, :], xc)
            for j in range(HG):
                vh = jnp.concatenate([vt[j * DH:(j + 1) * DH], vtail], axis=0).astype(BF16)
                for c in range(TQ // CK):
                    vt_s[i * (TQ // CK) + c, (g * HG + j) * HP:(g * HG + j + 1) * HP, :] = (
                        vh[:, c * CK:(c + 1) * CK])

    def proj_h(c0):
        x32 = xt_s[:, pl.ds(c0, 128)].astype(F32)
        r, mr = _ln_stats(x32)
        ln = (x32 * r - mr).astype(BF16)
        h_s[:, pl.ds(c0 + HALO, 128)] = _gelu(_dot_tn(w1_s[...], ln)).astype(BF16)

    cp["wv"].wait()
    wkvt_s[voff:voff + D, :] = wqkv_s[:, 2 * D:3 * D].T
    cp["x0"].wait()
    proj_v(0)
    cp["x1"].wait()
    cp["wk"].wait()
    for name in OPT["dma1"].split(","):
        cp[name].start()
    wkvt_s[0:voff, :] = wqkv_s[:, KLO:2 * D].T
    proj_v(1)
    proj_k(0)
    proj_k(1)
    for name in ("x2", "x3", "wq", "w1", "gw", "wo"):
        cp[name].wait()
    proj_k(2)
    wqt = wqkv_s[:, 0:KLO + 128].T
    for g in range(NG):
        wqt_s[g] = wqt[g * GW:(g + 1) * GW]
    proj_k(3)
    gw_s[...] = jnp.broadcast_to(gw_ref[...].astype(F32).reshape(1, D), (128, D)).T
    proj_h(0)
    proj_v(2)
    wot_s[...] = wo_s[...].T
    proj_v(3)
    for name in ("w2", "w3", "w4"):
        cp[name].wait()

    sb = (s_a, s_b)
    mb = (m_a, m_b)
    row = lax.broadcasted_iota(jnp.int32, (128, TQ), 0)

    def stage(nxt, cur, par, fill):
        if nxt is not None:
            u1, g1, j1 = nxt
            qg = qt_s[u1]
            qg = jnp.where((row >= DH * j1) & (row < DH * (j1 + 1)), qg, jnp.zeros_like(qg))
        if cur is not None:
            blk, j = cur
            hrow = pl.multiple_of(((blk % NG) * HG + j) * HP, HP)
            m = mb[1 - par][...]
        mx = None
        acc = None
        for c in range(NC):
            sl = pl.ds(c * CK, CK)
            if nxt is not None:
                s = _dot(k_s[g1, sl, :], qg)
                sb[par][sl, :] = s
                cm = jnp.max(s.reshape(CK // 8, 8, TQ), axis=0)
                mx = cm if mx is None else jnp.maximum(mx, cm)
            if cur is not None:
                p = jnp.exp2(sb[1 - par][sl, :] - m).astype(BF16)
                o = _dot(vt_s[c, pl.ds(hrow, HP), :], p)
                acc = o if acc is None else acc + o
                if c == NC - 1:
                    inv = 1.0 / acc[DH:DH + 1, :]
                    ot_s[blk, j * DH:(j + 1) * DH, :] = (acc * inv)[0:DH]
            for f in fill.get(c, []):
                f()
        if nxt is not None:
            mb[par][...] = jnp.max(mx, axis=0, keepdims=True)

    nsteps = UG * HG

    def main_body(it, carry):
        c0 = pl.multiple_of(it * TB, TB)
        st = {}

        def proj_q(u):
            blk = it * UG + u
            q0 = pl.multiple_of((blk // NG) * TQ, TQ)
            q = _dot(wqt_s[blk % NG], xt_s[:, pl.ds(q0, TQ)]) * qscale
            qt_s[u, 0:GW, :] = q.astype(BF16)

        def mix_h(k):
            proj_h(pl.multiple_of(c0 + (k + 1) * 128, 128))

        def mix_a():
            x32 = xt_s[:, pl.ds(c0, TB)].astype(F32)
            parts = []
            for g, sh in enumerate((-1, 1, -2, 2)):
                hw = h_s[g * C:(g + 1) * C, pl.ds(c0, TB + 2 * HALO)]
                parts.append(hw[:, HALO + sh:HALO + sh + TB])
            hs = jnp.concatenate(parts, axis=0)
            x1 = x32 + _dot_tn(w2_s[...], hs)
            bb_s[:, pl.ds(c0, TB)] = x1
            r, mr = _ln_stats(x1)
            st["ln"] = (bb_s[:, pl.ds(c0, TB)] * r - mr).astype(BF16)
            gw = jnp.concatenate([gw_s[...]] * (TB // 128), axis=1)
            gate_s[:, pl.ds(c0, TB)] = jax.nn.sigmoid(jnp.sum(x32 * gw, axis=0, keepdims=True))

        def mix_b(lo, hi):
            g_s[lo:hi, :] = _gelu(_dot_tn(w3_s[:, lo:hi], st["ln"])).astype(BF16)

        def mix_c(lo, hi):
            b = bb_s[lo:hi, pl.ds(c0, TB)] + _dot(w4t_s[lo:hi, :], g_s[...])
            bb_s[lo:hi, pl.ds(c0, TB)] = (1.0 - gate_s[:, pl.ds(c0, TB)]) * b

        slots = [s.split(",") if s else [] for s in OPT["plan"].split("|")]
        assert len(slots) == nsteps + 2
        names = [e.split("@")[0] for s in slots for e in s]
        nb, nc = names.count("b"), names.count("c")
        bb = [((FF // 256) * k // nb) * 256 for k in range(nb + 1)]
        cb = [((D // 16) * k // nc) * 16 for k in range(nc + 1)]
        kb = kc = 0
        fills = []
        for s in slots:
            fill = {}
            for e in s:
                name, _, at = e.partition("@")
                if name == "b":
                    f = functools.partial(mix_b, bb[kb], bb[kb + 1])
                    kb += 1
                elif name == "c":
                    f = functools.partial(mix_c, cb[kc], cb[kc + 1])
                    kc += 1
                elif name == "a":
                    f = mix_a
                else:
                    f = functools.partial(dict(q=proj_q, h=mix_h)[name[0]], int(name[1]))
                fill.setdefault(int(at) if at else NC - 1, []).append(f)
            fills.append(fill)

        for f in fills[0].get(NC - 1, []):
            f()
        for t in range(nsteps + 1):
            nxt = cur = None
            if t < nsteps:
                u, j = divmod(t, HG)
                nxt = (u, (it * UG + u) % NG, j)
            if t > 0:
                u, j = divmod(t - 1, HG)
                cur = (it * UG + u, j)
            stage(nxt, cur, t % 2, fills[t + 1])
        return carry

    lax.fori_loop(0, NIT, main_body, 0)

    for i in range(NQ):
        ot = jnp.concatenate([ot_s[i * NG + g] for g in range(NG)], axis=0).astype(BF16)
        for r in range(NOS):
            rows = slice(r * RO, (r + 1) * RO)
            a = _dot(wot_s[rows, :], ot)
            out_s[i, rows, :] = (gate_s[:, i * TQ:(i + 1) * TQ] * a
                                 + bb_s[rows, i * TQ:(i + 1) * TQ]).astype(out_s.dtype)
            out_copy(i, r).start()
    for i in range(NQ):
        for r in range(NOS):
            out_copy(i, r).wait()


@jax.jit
def pallas_gated_mix__mha_block__mixer_s_mlp__prompt_kernel(
    A_x: jax.Array,
    A_wqkv: jax.Array,
    A_wo: jax.Array,
    B_x: jax.Array,
    B_w1: jax.Array,
    B_w2: jax.Array,
    B_w3: jax.Array,
    B_w4: jax.Array,
    gate_w: jax.Array,
):
    del B_x
    B, S, D = A_x.shape
    assert B == 1 and S == 4 * TQ
    FF = B_w3.shape[1]
    NQ = S // TQ
    GW = D // NG
    TB = S // (NQ * NG // UG)
    KLO = (D // 128) * 128

    scratch = [
        pltpu.VMEM((D,), BF16),
        pltpu.VMEM((D, S + HALO), BF16),
        pltpu.VMEM((D, 3 * D), BF16),
        pltpu.VMEM((D, D), BF16),
        pltpu.VMEM((D, D), BF16),
        pltpu.VMEM((D, D), BF16),
        pltpu.VMEM((D, FF), BF16),
        pltpu.VMEM((D, FF), BF16),
        pltpu.VMEM((NQ, D, TQ), BF16),
        pltpu.SemaphoreType.DMA((9,)),
        pltpu.SemaphoreType.DMA((NQ,)),
        pltpu.SemaphoreType.DMA((NQ * NOS,)),
        pltpu.VMEM((3 * D - KLO, D), BF16),
        pltpu.VMEM((NG, GW, D), BF16),
        pltpu.VMEM((D, D), BF16),
        pltpu.VMEM((D, 128), F32),
        pltpu.VMEM((UG, 128, TQ), BF16),
        pltpu.VMEM((NG, S, 128), BF16),
        pltpu.VMEM((S // CK, H * HP, CK), BF16),
        pltpu.VMEM((NQ * NG, GW, TQ), F32),
        pltpu.VMEM((S, TQ), F32),
        pltpu.VMEM((S, TQ), F32),
        pltpu.VMEM((1, TQ), F32),
        pltpu.VMEM((1, TQ), F32),
        pltpu.VMEM((D, S + 2 * HALO), BF16),
        pltpu.VMEM((FF, TB), BF16),
        pltpu.VMEM((D, S), F32),
        pltpu.VMEM((1, S), F32),
    ]
    anyspec = pl.BlockSpec(memory_space=pl.ANY)
    out_t = pl.pallas_call(
        functools.partial(_kernel, S=S, D=D, FF=FF),
        out_shape=jax.ShapeDtypeStruct((D, S), A_x.dtype),
        in_specs=[anyspec] * 8,
        out_specs=anyspec,
        scratch_shapes=scratch,
        compiler_params=pltpu.CompilerParams(vmem_limit_bytes=64 * 1024 * 1024),
        name="gated_mix",
    )(A_x.reshape(S, D).T, A_wqkv, A_wo, B_w1, B_w2, B_w3, B_w4.T, gate_w)
    return out_t.T.reshape(B, S, D)
```

```python
import functools
import math

import jax
import jax.numpy as jnp
from jax import lax
import jax.experimental.pallas as pl
import jax.experimental.pallas.tpu as pltpu

F32 = jnp.float32
BF16 = jnp.bfloat16

H = 16
HG = 4
NG = H // HG
HP = 32
TQ = 512
CK = 128
EPS = 1e-5
HALO = 128
UG = 2
NOS = 4

OPT = dict(
    last_rows=(0, 160, 320, 416, 448),
    xb=(0, 2, 6, 10, 16),
    dma0="wv,x0,x1,wk,x2,x3,wq,w1,gw",
    p1="Wwv,Twv,Wx0,v0-2,Wx1,v2-6,"
       "Wwk,Wx2,Swo,Sw2,Sw3,Sw4,Twk,v6-10g01,k0-4,k4-8,v6-10g23,"
       "Wx3,Wwq,Ww1,Wgw,Wwo,k8-12,Twq,k12-16,Tgw,h,v10-12,Two,v12-16,"
       "Ww2,Ww3,Ww4",
    plan="q0,q1|h0@3,h1@9,a|b|b|b|b|b|b,b|c|c@2,c@5,c@8,c@11,c@14,c",
)

_TN = (((0,), (0,)), ((), ()))


def _dot(a, b):
    return jnp.dot(a, b, preferred_element_type=F32)


def _dot_tn(a, b):
    return lax.dot_general(a, b, _TN, preferred_element_type=F32)


def _gelu(x):
    c = math.sqrt(2.0 / math.pi)
    hx = 0.5 * x
    return hx + hx * jnp.tanh(x * (c + (c * 0.044715) * (x * x)))


def _ln_stats(x):
    n = x.shape[0]
    p = x[0:1, :]
    d = x - p
    s1 = jnp.sum(d, axis=0, keepdims=True) * (1.0 / n)
    s2 = jnp.sum(d * d, axis=0, keepdims=True) * (1.0 / n)
    v = jnp.maximum(s2 - s1 * s1, 0.0)
    r = lax.rsqrt(v + EPS)
    return r, (p + s1) * r


def _kernel(xt_hbm, wqkv_hbm, wo_hbm, w1_hbm, w2_hbm, w3_hbm, w4t_hbm, gw_hbm,
            out_hbm,
            gw_ref, xt_s, wqkv_s, w1_s, w2_s, wo_s, w3_s, w4t_s, out_s, sem_in, sem_x, sem_out,
            wkvt_s, wqt_s, wot_s, gw_s,
            qt_s, k_s, vt_s, ot_s, s_a, s_b, m_a, m_b, h_s, g_s, bb_s, gate_s,
            *, S, D, FF):
    DH = D // H
    GW = HG * DH
    NQ = S // TQ
    NC = S // CK
    qscale = (DH ** -0.5) * math.log2(math.e)
    NIT = NQ * NG // UG
    TB = S // NIT
    RO = D // NOS
    KLO = (D // 128) * 128
    C = D // 4

    def out_rows(i):
        return OPT["last_rows"] if i == NQ - 1 else tuple(range(0, D + 1, RO))

    def out_copy(i, r):
        lo, hi = out_rows(i)[r:r + 2]
        return pltpu.make_async_copy(out_s.at[i, pl.ds(lo, hi - lo)],
                                     out_hbm.at[pl.ds(lo, hi - lo), pl.ds(i * TQ, TQ)],
                                     sem_out.at[i * NOS + r])

    def col_copy(src, dst, lo, hi, sem):
        return pltpu.make_async_copy(src.at[:, lo:hi], dst.at[:, lo:hi], sem)

    cp = dict(
        wk=col_copy(wqkv_hbm, wqkv_s, KLO, 2 * D, sem_in.at[0]),
        wv=col_copy(wqkv_hbm, wqkv_s, 2 * D, 3 * D, sem_in.at[1]),
        wq=col_copy(wqkv_hbm, wqkv_s, 0, KLO, sem_in.at[2]),
        w1=pltpu.make_async_copy(w1_hbm, w1_s, sem_in.at[3]),
        w3=pltpu.make_async_copy(w3_hbm, w3_s, sem_in.at[4]),
        w2=pltpu.make_async_copy(w2_hbm, w2_s, sem_in.at[5]),
        wo=pltpu.make_async_copy(wo_hbm, wo_s, sem_in.at[6]),
        w4=pltpu.make_async_copy(w4t_hbm, w4t_s, sem_in.at[7]),
        gw=pltpu.make_async_copy(gw_hbm, gw_ref, sem_in.at[8]),
    )
    xb = OPT["xb"]
    for i in range(len(xb) - 1):
        cp["x%d" % i] = col_copy(xt_hbm, xt_s, xb[i] * 128, xb[i + 1] * 128, sem_x.at[i])

    for name in OPT["dma0"].split(","):
        cp[name].start()
    h_s[:, 0:HALO] = jnp.zeros((D, HALO), BF16)
    xt_s[:, S:S + HALO] = jnp.zeros((D, HALO), BF16)
    for ref in (s_a, s_b):
        ref[0:8, :] = jnp.zeros((8, TQ), F32)
    for ref in (m_a, m_b):
        ref[...] = jnp.zeros_like(ref)
    for u in range(UG):
        qt_s[u, GW:128, :] = jnp.zeros((128 - GW, TQ), BF16)

    koff = D - KLO
    voff = 2 * D - KLO

    def proj_k(lo, hi, groups=range(NG)):
        xc = xt_s[:, lo:hi]
        zpad = jnp.zeros((128 - GW, hi - lo), BF16)
        for g in groups:
            kt = _dot(wkvt_s[koff + g * GW:koff + (g + 1) * GW, :], xc)
            kt = jnp.concatenate([kt.astype(BF16), zpad], axis=0)
            k_s[g, lo:hi, :] = kt.T

    def proj_v(lo, hi, groups=range(NG)):
        xc = xt_s[:, lo:hi]
        rowv = lax.broadcasted_iota(jnp.int32, (HP - DH, hi - lo), 0)
        vtail = jnp.where(rowv == 0, 1.0, 0.0).astype(F32)
        for g in groups:
            vt = _dot(wkvt_s[voff + g * GW:voff + (g + 1) * GW, :], xc)
            for j in range(HG):
                vh = jnp.concatenate([vt[j * DH:(j + 1) * DH], vtail], axis=0).astype(BF16)
                for c in range((hi - lo) // CK):
                    vt_s[lo // CK + c, (g * HG + j) * HP:(g * HG + j + 1) * HP, :] = (
                        vh[:, c * CK:(c + 1) * CK])

    def proj_h(c0):
        x32 = xt_s[:, pl.ds(c0, 128)].astype(F32)
        r, mr = _ln_stats(x32)
        ln = (x32 * r - mr).astype(BF16)
        h_s[:, pl.ds(c0 + HALO, 128)] = _gelu(_dot_tn(w1_s[...], ln)).astype(BF16)

    def t_wv():
        wkvt_s[voff:voff + D, :] = wqkv_s[:, 2 * D:3 * D].T

    def t_wk():
        wkvt_s[0:voff, :] = wqkv_s[:, KLO:2 * D].T

    def t_wq():
        wqt = wqkv_s[:, 0:KLO + 128].T
        for g in range(NG):
            wqt_s[g] = wqt[g * GW:(g + 1) * GW]

    def t_gw():
        gw_s[...] = jnp.broadcast_to(gw_ref[...].astype(F32).reshape(1, D), (128, D)).T

    def t_wo():
        wot_s[...] = wo_s[...].T

    for op in OPT["p1"].split(","):
        if op[0] == "W":
            cp[op[1:]].wait()
        elif op[0] == "S":
            cp[op[1:]].start()
        elif op[0] == "T":
            dict(wv=t_wv, wk=t_wk, wq=t_wq, gw=t_gw, wo=t_wo)[op[1:]]()
        elif op == "h":
            proj_h(0)
        else:
            rng, _, gs = op[1:].partition("g")
            lo, hi = (int(v) * 128 for v in rng.split("-"))
            groups = [int(ch) for ch in gs] if gs else range(NG)
            dict(k=proj_k, v=proj_v)[op[0]](lo, hi, groups)

    sb = (s_a, s_b)
    mb = (m_a, m_b)
    row = lax.broadcasted_iota(jnp.int32, (128, TQ), 0)

    def stage(nxt, cur, par, fill):
        if nxt is not None:
            u1, g1, j1 = nxt
            qg = qt_s[u1]
            qg = jnp.where((row >= DH * j1) & (row < DH * (j1 + 1)), qg, jnp.zeros_like(qg))
        if cur is not None:
            blk, j = cur
            hrow = pl.multiple_of(((blk % NG) * HG + j) * HP, HP)
            m = mb[1 - par][...]
        mx = None
        acc = None
        for c in range(NC):
            sl = pl.ds(c * CK, CK)
            if nxt is not None:
                s = _dot(k_s[g1, sl, :], qg)
                sb[par][sl, :] = s
                cm = jnp.max(s.reshape(CK // 8, 8, TQ), axis=0)
                mx = cm if mx is None else jnp.maximum(mx, cm)
            if cur is not None:
                p = jnp.exp2(sb[1 - par][sl, :] - m).astype(BF16)
                o = _dot(vt_s[c, pl.ds(hrow, HP), :], p)
                acc = o if acc is None else acc + o
                if c == NC - 1:
                    inv = 1.0 / acc[DH:DH + 1, :]
                    ot_s[blk, j * DH:(j + 1) * DH, :] = (acc * inv)[0:DH]
            for f in fill.get(c, []):
                f()
        if nxt is not None:
            mb[par][...] = jnp.max(mx, axis=0, keepdims=True)

    nsteps = UG * HG

    def main_body(it, carry):
        c0 = pl.multiple_of(it * TB, TB)
        st = {}

        def proj_q(u):
            blk = it * UG + u
            q0 = pl.multiple_of((blk // NG) * TQ, TQ)
            q = _dot(wqt_s[blk % NG], xt_s[:, pl.ds(q0, TQ)]) * qscale
            qt_s[u, 0:GW, :] = q.astype(BF16)

        def mix_h(k):
            proj_h(pl.multiple_of(c0 + (k + 1) * 128, 128))

        def mix_a():
            x32 = xt_s[:, pl.ds(c0, TB)].astype(F32)
            parts = []
            for g, sh in enumerate((-1, 1, -2, 2)):
                hw = h_s[g * C:(g + 1) * C, pl.ds(c0, TB + 2 * HALO)]
                parts.append(hw[:, HALO + sh:HALO + sh + TB])
            hs = jnp.concatenate(parts, axis=0)
            x1 = x32 + _dot_tn(w2_s[...], hs)
            bb_s[:, pl.ds(c0, TB)] = x1
            r, mr = _ln_stats(x1)
            st["ln"] = (bb_s[:, pl.ds(c0, TB)] * r - mr).astype(BF16)
            gw = jnp.concatenate([gw_s[...]] * (TB // 128), axis=1)
            gate_s[:, pl.ds(c0, TB)] = jax.nn.sigmoid(jnp.sum(x32 * gw, axis=0, keepdims=True))

        def mix_b(lo, hi):
            g_s[lo:hi, :] = _gelu(_dot_tn(w3_s[:, lo:hi], st["ln"])).astype(BF16)

        def mix_c(lo, hi):
            b = bb_s[lo:hi, pl.ds(c0, TB)] + _dot(w4t_s[lo:hi, :], g_s[...])
            bb_s[lo:hi, pl.ds(c0, TB)] = (1.0 - gate_s[:, pl.ds(c0, TB)]) * b

        slots = [s.split(",") if s else [] for s in OPT["plan"].split("|")]
        assert len(slots) == nsteps + 2
        names = [e.split("@")[0] for s in slots for e in s]
        nb, nc = names.count("b"), names.count("c")
        bb = [((FF // 256) * k // nb) * 256 for k in range(nb + 1)]
        cb = [((D // 16) * k // nc) * 16 for k in range(nc + 1)]
        kb = kc = 0
        fills = []
        for s in slots:
            fill = {}
            for e in s:
                name, _, at = e.partition("@")
                if name == "b":
                    f = functools.partial(mix_b, bb[kb], bb[kb + 1])
                    kb += 1
                elif name == "c":
                    f = functools.partial(mix_c, cb[kc], cb[kc + 1])
                    kc += 1
                elif name == "a":
                    f = mix_a
                else:
                    f = functools.partial(dict(q=proj_q, h=mix_h)[name[0]], int(name[1]))
                fill.setdefault(int(at) if at else NC - 1, []).append(f)
            fills.append(fill)

        for f in fills[0].get(NC - 1, []):
            f()
        for t in range(nsteps + 1):
            nxt = cur = None
            if t < nsteps:
                u, j = divmod(t, HG)
                nxt = (u, (it * UG + u) % NG, j)
            if t > 0:
                u, j = divmod(t - 1, HG)
                cur = (it * UG + u, j)
            stage(nxt, cur, t % 2, fills[t + 1])
        return carry

    lax.fori_loop(0, NIT, main_body, 0)

    for i in range(NQ):
        ot = jnp.concatenate([ot_s[i * NG + g] for g in range(NG)], axis=0).astype(BF16)
        for r in range(NOS):
            rows = slice(*out_rows(i)[r:r + 2])
            a = _dot(wot_s[rows, :], ot)
            out_s[i, rows, :] = (gate_s[:, i * TQ:(i + 1) * TQ] * a
                                 + bb_s[rows, i * TQ:(i + 1) * TQ]).astype(out_s.dtype)
            out_copy(i, r).start()
    for i in range(NQ):
        for r in range(NOS):
            out_copy(i, r).wait()


@jax.jit
def pallas_gated_mix__mha_block__mixer_s_mlp__prompt_kernel(
    A_x: jax.Array,
    A_wqkv: jax.Array,
    A_wo: jax.Array,
    B_x: jax.Array,
    B_w1: jax.Array,
    B_w2: jax.Array,
    B_w3: jax.Array,
    B_w4: jax.Array,
    gate_w: jax.Array,
):
    del B_x
    B, S, D = A_x.shape
    assert B == 1 and S == 4 * TQ
    FF = B_w3.shape[1]
    NQ = S // TQ
    GW = D // NG
    TB = S // (NQ * NG // UG)
    KLO = (D // 128) * 128

    scratch = [
        pltpu.VMEM((D,), BF16),
        pltpu.VMEM((D, S + HALO), BF16),
        pltpu.VMEM((D, 3 * D), BF16),
        pltpu.VMEM((D, D), BF16),
        pltpu.VMEM((D, D), BF16),
        pltpu.VMEM((D, D), BF16),
        pltpu.VMEM((D, FF), BF16),
        pltpu.VMEM((D, FF), BF16),
        pltpu.VMEM((NQ, D, TQ), BF16),
        pltpu.SemaphoreType.DMA((9,)),
        pltpu.SemaphoreType.DMA((len(OPT['xb']) - 1,)),
        pltpu.SemaphoreType.DMA((NQ * NOS,)),
        pltpu.VMEM((3 * D - KLO, D), BF16),
        pltpu.VMEM((NG, GW, D), BF16),
        pltpu.VMEM((D, D), BF16),
        pltpu.VMEM((D, 128), F32),
        pltpu.VMEM((UG, 128, TQ), BF16),
        pltpu.VMEM((NG, S, 128), BF16),
        pltpu.VMEM((S // CK, H * HP, CK), BF16),
        pltpu.VMEM((NQ * NG, GW, TQ), F32),
        pltpu.VMEM((S, TQ), F32),
        pltpu.VMEM((S, TQ), F32),
        pltpu.VMEM((1, TQ), F32),
        pltpu.VMEM((1, TQ), F32),
        pltpu.VMEM((D, S + 2 * HALO), BF16),
        pltpu.VMEM((FF, TB), BF16),
        pltpu.VMEM((D, S), F32),
        pltpu.VMEM((1, S), F32),
    ]
    anyspec = pl.BlockSpec(memory_space=pl.ANY)
    out_t = pl.pallas_call(
        functools.partial(_kernel, S=S, D=D, FF=FF),
        out_shape=jax.ShapeDtypeStruct((D, S), A_x.dtype),
        in_specs=[anyspec] * 8,
        out_specs=anyspec,
        scratch_shapes=scratch,
        compiler_params=pltpu.CompilerParams(vmem_limit_bytes=64 * 1024 * 1024),
        name="gated_mix",
    )(A_x.reshape(S, D).T, A_wqkv, A_wo, B_w1, B_w2, B_w3, B_w4.T, gate_w)
    return out_t.T.reshape(B, S, D)
```
